```python
import os as _os
_os.environ.setdefault("JAX_PLATFORMS", "cpu")
import jax
import jax.numpy as jnp

def _softmax(x, axis=-1):
    return jax.nn.softmax(x, axis=axis)
def _gelu(x):
    return jax.nn.gelu(x, approximate=True)
def _silu(x):
    return jax.nn.silu(x)
def _sigmoid(x):
    return jax.nn.sigmoid(x)
def _layernorm(x, axis=-1, eps=1e-5):
    m = jnp.mean(x, axis=axis, keepdims=True)
    v = jnp.var(x, axis=axis, keepdims=True)
    return (x - m) / jnp.sqrt(v + eps)
def _scatter_add(tgt, idx, src, axis=0):
    return tgt.at[idx].add(src)
def _segment_sum(src, seg, n):
    return jax.ops.segment_sum(src, seg, n)
class _Rng:
    def __init__(self, key):
        self._k = key
    def _next(self):
        self._k, sub = jax.random.split(self._k)
        return sub
    def normal(self, shape):
        return jax.random.normal(self._next(), shape, dtype=jnp.bfloat16)
    def randint(self, lo, hi, shape):
        return jax.random.randint(self._next(), shape, lo, hi, dtype=jnp.int32)
    def uniform(self, shape, lo=0.0, hi=1.0):
        return jax.random.uniform(self._next(), shape, jnp.bfloat16, lo, hi)
    def permutation(self, n):
        return jax.random.permutation(self._next(), n)


kernel_name = 'concat_heads__mha_block_cached__mha_block_cached__near_ridge'

def setup_inputs():
    _rng = _Rng(jax.random.key(int.from_bytes(__import__("os").urandom(4), "little")))
    _w = (lambda a: (lambda t: t.astype(jnp.bfloat16) if jnp.issubdtype(t.dtype, jnp.floating) else t)(jnp.asarray(a)))
    def _A_setup():
        B, Sq, D = 16, 192, 512
        H, Sk, Dh = 32, 512, 128
        return {
            "x": _w((lambda *s: _rng.normal(s) * 0.8)(B, Sq, D)),
            "k_cache": _w((lambda *s: _rng.normal(s) * 0.8)(B, H, Sk, Dh)),
            "v_cache": _w((lambda *s: _rng.normal(s) * 0.05)(B, H, Sk, Dh)),
            "wq": _w((lambda *s: _rng.normal(s) * 0.8)(D, H * Dh) * (D ** -0.5)),
            "wo": _w((lambda *s: _rng.normal(s) * 0.05)(H * Dh, D) * ((H * Dh) ** -0.5)),
        }
    _A_in = _A_setup()

    def _B_setup():
        B, Sq, D = 16, 192, 512
        H, Sk, Dh = 32, 512, 128
        return {
            "x": _w((lambda *s: _rng.normal(s) * 0.8)(B, Sq, D)),
            "k_cache": _w((lambda *s: _rng.normal(s) * 0.8)(B, H, Sk, Dh)),
            "v_cache": _w((lambda *s: _rng.normal(s) * 0.05)(B, H, Sk, Dh)),
            "wq": _w((lambda *s: _rng.normal(s) * 0.8)(D, H * Dh) * (D ** -0.5)),
            "wo": _w((lambda *s: _rng.normal(s) * 0.05)(H * Dh, D) * ((H * Dh) ** -0.5)),
        }
    _B_in = _B_setup()

    return {
        "A_x": _A_in["x"],
        "A_k_cache": _A_in["k_cache"],
        "A_v_cache": _A_in["v_cache"],
        "A_wq": _A_in["wq"],
        "A_wo": _A_in["wo"],
        "B_x": _B_in["x"],
        "B_k_cache": _B_in["k_cache"],
        "B_v_cache": _B_in["v_cache"],
        "B_wq": _B_in["wq"],
        "B_wo": _B_in["wo"],
    }

def reference(A_x, A_k_cache, A_v_cache, A_wq, A_wo, B_x, B_k_cache, B_v_cache, B_wq, B_wo):
    def _A_ref(x, k_cache, v_cache, wq, wo):
        B, Sq, D = x.shape
        H, Dh = 32, 128
        q = (lambda x, *d: x.transpose(*d))((x @ wq).reshape(B, Sq, H, Dh), 0, 2, 1, 3)
        scores = jnp.einsum("bhqd,bhkd->bhqk", q, k_cache) * (Dh ** -0.5)
        p = _softmax(scores, axis=-1)
        o = jnp.einsum("bhqk,bhkd->bhqd", p, v_cache)
        return (lambda x, *d: x.transpose(*d))(o, 0, 2, 1, 3).reshape(B, Sq, H * Dh) @ wo

    def _B_ref(x, k_cache, v_cache, wq, wo):
        B, Sq, D = x.shape
        H, Dh = 32, 128
        q = (lambda x, *d: x.transpose(*d))((x @ wq).reshape(B, Sq, H, Dh), 0, 2, 1, 3)
        scores = jnp.einsum("bhqd,bhkd->bhqk", q, k_cache) * (Dh ** -0.5)
        p = _softmax(scores, axis=-1)
        o = jnp.einsum("bhqk,bhkd->bhqd", p, v_cache)
        return (lambda x, *d: x.transpose(*d))(o, 0, 2, 1, 3).reshape(B, Sq, H * Dh) @ wo

    a = _A_ref(A_x, A_k_cache, A_v_cache, A_wq, A_wo)
    b = _B_ref(B_x, B_k_cache, B_v_cache, B_wq, B_wo)
    return jnp.concatenate([a, b], axis=-1)
```

```python
import functools
import jax
import jax.numpy as jnp
from jax import lax
import jax.experimental.pallas as pl
import jax.experimental.pallas.tpu as pltpu

B, SQ, D = 16, 192, 512
H, SK, DH = 32, 512, 128
LOG2E = 1.4426950408889634
QSCALE = (DH ** -0.5) * LOG2E
F32 = jnp.float32
BF16 = jnp.bfloat16


def _kernel(xa, ka, va, wqa, woa, xb, kb, vb, wqb, wob, o_hbm,
            x_buf, k_buf, v_buf, wq_buf, wo_buf, acc_ref, o_buf,
            x_sem, k_sem, v_sem, wq_sem, wo_sem, o_sem, *, hg):
    ng = H // hg
    g = pl.program_id(0)
    b = pl.program_id(1)
    slot = lax.rem(b, 2) if False else jnp.bitwise_and(b, 1)
    gslot = jnp.bitwise_and(g, 1)
    xs, ks, vs, wqs, wos = (xa, xb), (ka, kb), (va, vb), (wqa, wqb), (woa, wob)

    def kv_copies(gg, bb, sl):
        cps = []
        for p in range(2):
            cps.append(pltpu.make_async_copy(xs[p].at[bb], x_buf.at[sl, p], x_sem.at[sl, p]))
            cps.append(pltpu.make_async_copy(ks[p].at[bb, pl.ds(gg * hg, hg)], k_buf.at[sl, p], k_sem.at[sl, p]))
            cps.append(pltpu.make_async_copy(vs[p].at[bb, pl.ds(gg * hg, hg)], v_buf.at[sl, p], v_sem.at[sl, p]))
        return cps

    def wq_copy(gg, sl, p):
        return pltpu.make_async_copy(
            wqs[p].at[:, pl.ds(pl.multiple_of(gg * (hg * DH), hg * DH), hg * DH)], wq_buf.at[sl, p], wq_sem.at[sl, p])

    def wo_copy(gg, sl, p):
        return pltpu.make_async_copy(
            wos[p].at[pl.ds(pl.multiple_of(gg * (hg * DH), hg * DH), hg * DH), :], wo_buf.at[sl, p], wo_sem.at[sl, p])

    def o_copy(bb, sl):
        return pltpu.make_async_copy(o_buf.at[sl], o_hbm.at[bb], o_sem.at[sl])

    first = jnp.logical_and(g == 0, b == 0)

    @pl.when(first)
    def _():
        cps = kv_copies(0, 0, 0)
        cps[0].start(); wq_copy(0, 0, 0).start(); cps[1].start(); cps[2].start(); wo_copy(0, 0, 0).start()
        cps[3].start(); wq_copy(0, 0, 1).start(); cps[4].start(); cps[5].start(); wo_copy(0, 0, 1).start()
        for c in kv_copies(0, 1, 1):
            c.start()

    for c in kv_copies(g, b, slot):
        c.wait()

    @pl.when(b == 0)
    def _():
        for p in range(2):
            wq_copy(g, gslot, p).wait()
            wo_copy(g, gslot, p).wait()

    heads = [(p, h) for p in range(2) for h in range(hg)]
    n = len(heads)
    q, s, o = {}, {}, {}

    def qproj(i):
        p, h = heads[i]
        qq = jnp.dot(x_buf[slot, p], wq_buf[gslot, p, :, h * DH:(h + 1) * DH], preferred_element_type=F32)
        q[i] = (qq * QSCALE).astype(BF16)

    def qk(i):
        p, h = heads[i]
        s[i] = jax.lax.dot_general(q.pop(i), k_buf[slot, p, h], (((1,), (1,)), ((), ())),
                                   preferred_element_type=F32)

    def pv(i):
        p, h = heads[i]
        sc = s.pop(i)
        m = jnp.max(sc, axis=-1, keepdims=True)
        e = jnp.exp2(sc - m)
        l = jnp.sum(e, axis=-1, keepdims=True)
        oo = jnp.dot(e.astype(BF16), v_buf[slot, p, h], preferred_element_type=F32)
        r = pl.reciprocal(l, approx=True)
        r = r * (2.0 - l * r)
        o[i] = (oo * r).astype(BF16)

    def out(i):
        p, h = heads[i]
        d = jnp.dot(o.pop(i), wo_buf[gslot, p, h * DH:(h + 1) * DH, :], preferred_element_type=F32)
        prev = acc_ref[b, :, p * D:(p + 1) * D]
        if h == 0:
            prev = jnp.where(g > 0, prev, 0.0)
        acc_ref[b, :, p * D:(p + 1) * D] = prev + d

    qproj(0)
    for i in range(n):
        qk(i)
        if i + 1 < n:
            qproj(i + 1)
        if i >= 1:
            out(i - 1)
        pv(i)
    out(n - 1)

    b2 = b + 2
    wrap = b2 >= B
    g2 = jnp.where(wrap, g + 1, g)
    b2 = jnp.where(wrap, b2 - B, b2)

    @pl.when(g2 < ng)
    def _():
        for c in kv_copies(g2, b2, slot):
            c.start()

    for j, (fn, p) in enumerate(((wq_copy, 0), (wo_copy, 0), (wq_copy, 1), (wo_copy, 1))):
        @pl.when(jnp.logical_and(b == j + 1, g + 1 < ng))
        def _(fn=fn, p=p):
            fn(g + 1, 1 - gslot, p).start()

    @pl.when(g == ng - 1)
    def _():
        @pl.when(b >= 2)
        def _():
            o_copy(b - 2, slot).wait()

        o_buf[slot] = acc_ref[b].astype(BF16)
        o_copy(b, slot).start()

        @pl.when(b == B - 1)
        def _():
            o_copy(b - 1, 1 - slot).wait()
            o_copy(b, slot).wait()


def run(A_x, A_k_cache, A_v_cache, A_wq, A_wo, B_x, B_k_cache, B_v_cache, B_wq, B_wo, *, hg=8, nobc=True):
    ng = H // hg
    any_spec = pl.BlockSpec(memory_space=pl.ANY)
    return pl.pallas_call(
        functools.partial(_kernel, hg=hg),
        grid=(ng, B),
        in_specs=[any_spec] * 10,
        out_specs=any_spec,
        out_shape=jax.ShapeDtypeStruct((B, SQ, 2 * D), BF16),
        scratch_shapes=[
            pltpu.VMEM((2, 2, SQ, D), BF16),
            pltpu.VMEM((2, 2, hg, SK, DH), BF16),
            pltpu.VMEM((2, 2, hg, SK, DH), BF16),
            pltpu.VMEM((2, 2, D, hg * DH), BF16),
            pltpu.VMEM((2, 2, hg * DH, D), BF16),
            pltpu.VMEM((B, SQ, 2 * D), F32),
            pltpu.VMEM((2, SQ, 2 * D), BF16),
            pltpu.SemaphoreType.DMA((2, 2)),
            pltpu.SemaphoreType.DMA((2, 2)),
            pltpu.SemaphoreType.DMA((2, 2)),
            pltpu.SemaphoreType.DMA((2, 2)),
            pltpu.SemaphoreType.DMA((2, 2)),
            pltpu.SemaphoreType.DMA((2,)),
        ],
        compiler_params=pltpu.CompilerParams(
            dimension_semantics=("arbitrary", "arbitrary"),
            vmem_limit_bytes=100 * 1024 * 1024,
            disable_bounds_checks=nobc,
        ),
    )(A_x, A_k_cache, A_v_cache, A_wq, A_wo, B_x, B_k_cache, B_v_cache, B_wq, B_wo)


@jax.jit
def pallas_concat_heads__mha_block_cached__mha_block_cached__near_ridge_kernel(
        A_x, A_k_cache, A_v_cache, A_wq, A_wo, B_x, B_k_cache, B_v_cache, B_wq, B_wo):
    return run(A_x, A_k_cache, A_v_cache, A_wq, A_wo, B_x, B_k_cache, B_v_cache, B_wq, B_wo)
```

```python
import functools
import jax
import jax.numpy as jnp
from jax import lax
import jax.experimental.pallas as pl
import jax.experimental.pallas.tpu as pltpu

B, SQ, D = 16, 192, 512
H, SK, DH = 32, 512, 128
LOG2E = 1.4426950408889634
QSCALE = (DH ** -0.5) * LOG2E
F32 = jnp.float32
BF16 = jnp.bfloat16
NXS = 4


def _log2(n):
    assert n & (n - 1) == 0
    return n.bit_length() - 1


def _kernel(xa, ka, va, wqa, woa, xb, kb, vb, wqb, wob, o_hbm,
            x_buf, kv_buf, wq_buf, wo_buf, acc_ref, o_buf,
            u_sem, x_sem, kv_sem, wq_sem, wo_sem, o_sem, *, hg, nb, stages):
    ng = H // hg
    nbb = B // nb
    T = ng * nbb
    kw = len(stages)
    cpi = [hg // hc for hc in stages]
    uoff = [sum(cpi[:t]) for t in range(kw)]
    xs, ks, vs, wqs, wos = (xa, xb), (ka, kb), (va, vb), (wqa, wqb), (woa, wob)

    def split(t):
        return lax.shift_right_logical(t, _log2(nbb)), jnp.bitwise_and(t, nbb - 1)

    def wait_total(ref, sem):
        pltpu.make_async_copy(ref, ref, sem).wait()

    def start_x(bb, xslot, sem):
        for p in range(2):
            pltpu.make_async_copy(xs[p].at[pl.ds(bb * nb, nb)], x_buf.at[xslot, p], sem).start()

    def start_kv(gg, bb, sl, h0, nh, sem):
        for p in range(2):
            src = (pl.ds(bb * nb, nb), pl.ds(gg * hg + h0, nh))
            pltpu.make_async_copy(ks[p].at[src], kv_buf.at[sl, 2 * p, :, pl.ds(h0, nh)], sem).start()
            pltpu.make_async_copy(vs[p].at[src], kv_buf.at[sl, 2 * p + 1, :, pl.ds(h0, nh)], sem).start()

    def wq_copy(gg, sl, p, h0, nh, sem):
        return pltpu.make_async_copy(
            wqs[p].at[:, pl.ds(pl.multiple_of((gg * hg + h0) * DH, nh * DH), nh * DH)],
            wq_buf.at[sl, p, :, pl.ds(pl.multiple_of(h0 * DH, nh * DH), nh * DH)], sem)

    def wo_copy(gg, sl, p, h0, nh, sem):
        return pltpu.make_async_copy(
            wos[p].at[pl.ds(pl.multiple_of((gg * hg + h0) * DH, nh * DH), nh * DH), :],
            wo_buf.at[sl, p, pl.ds(pl.multiple_of(h0 * DH, nh * DH), nh * DH), :], sem)

    def o_copy(bb, sl):
        return pltpu.make_async_copy(o_buf.at[sl], o_hbm.at[pl.ds(bb * nb, nb)], o_sem.at[sl])

    def start_unit(t, r):
        hc = stages[t]
        sem = u_sem.at[uoff[t] + r]

        if isinstance(r, int):
            if r == 0:
                start_x(t, t % NXS, sem)
        else:
            @pl.when(r == 0)
            def _():
                start_x(t, t % NXS, sem)

        if t == 0:
            for p in range(2):
                wq_copy(0, 0, p, r * hc, hc, sem).start()
        start_kv(0, t, t % 2, r * hc, hc, sem)
        if t == 0:
            for p in range(2):
                wo_copy(0, 0, p, r * hc, hc, sem).start()

    def wait_unit(t, r):
        hc = stages[t]
        sem = u_sem.at[uoff[t] + r]

        @pl.when(r == 0)
        def _():
            wait_total(x_buf.at[t % NXS], sem)

        if t == 0:
            cols = pl.ds(pl.multiple_of(r * (hc * DH), hc * DH), hc * DH)
            wait_total(wq_buf.at[0, :, :, cols], sem)
            wait_total(wo_buf.at[0, :, cols, :], sem)
        wait_total(kv_buf.at[t % 2, :, :, pl.ds(r * hc, hc)], sem)

    def compute(xslot, slot, gslot, bb, h0, nh, first_acc, write_out):
        heads = [(p, h) for p in range(2) for h in range(nh)]
        n = len(heads)
        q, s, o = {}, {}, {}

        def wcols(h):
            if isinstance(h0, int):
                return slice((h0 + h) * DH, (h0 + h + 1) * DH)
            return pl.ds(pl.multiple_of((h0 + h) * DH, DH), DH)

        def qproj(i):
            p, h = heads[i]
            x = x_buf[xslot, p].reshape(nb * SQ, D)
            qq = jnp.dot(x, wq_buf[gslot, p, :, wcols(h)], preferred_element_type=F32)
            q[i] = (qq * QSCALE).astype(BF16)

        def qk(i, j):
            p, h = heads[i]
            s[i, j] = jax.lax.dot_general(q[i][j * SQ:(j + 1) * SQ], kv_buf[slot, 2 * p, j, h0 + h],
                                          (((1,), (1,)), ((), ())), preferred_element_type=F32)

        def pv(i, j):
            p, h = heads[i]
            sc = s.pop((i, j))
            m = jnp.max(sc, axis=-1, keepdims=True)
            e = jnp.exp2(sc - m)
            l = jnp.sum(e, axis=-1, keepdims=True)
            oo = jnp.dot(e.astype(BF16), kv_buf[slot, 2 * p + 1, j, h0 + h], preferred_element_type=F32)
            r = pl.reciprocal(l, approx=True)
            r = r * (2.0 - l * r)
            o[i, j] = (oo * r).astype(BF16)

        def out(i):
            p, h = heads[i]
            os_ = [o.pop((i, j)) for j in range(nb)]
            oc = jnp.concatenate(os_, axis=0) if nb > 1 else os_[0]
            d = jnp.dot(oc, wo_buf[gslot, p, wcols(h), :], preferred_element_type=F32)
            d = d.reshape(nb, SQ, D)
            prev = acc_ref[pl.ds(bb * nb, nb), :, p * D:(p + 1) * D]
            if h == 0:
                prev = jnp.where(first_acc, 0.0, prev)
            new = prev + d
            acc_ref[pl.ds(bb * nb, nb), :, p * D:(p + 1) * D] = new
            if write_out and h == nh - 1:
                o_buf[slot, :, :, p * D:(p + 1) * D] = new.astype(BF16)

        qproj(0)
        for i in range(n):
            for j in range(nb):
                qk(i, j)
            if i + 1 < n:
                qproj(i + 1)
            elif n > 1:
                out(i - 1)
            for j in range(nb):
                pv(i, j)
            if i != n - 2:
                out(i)

    def issue0(r, carry):
        start_unit(0, r)
        return carry

    lax.fori_loop(0, cpi[0], issue0, 0)

    for t in range(kw):
        hc = stages[t]

        def chunk(r, carry, t=t, hc=hc):
            wait_unit(t, r)
            compute(t % NXS, t % 2, 0, t, r * hc, hc, r == 0, False)

            t2 = t + 2

            def refill(rr):
                if t2 < kw:
                    ratio = stages[t2] // hc
                    kv_s = u_sem.at[uoff[t2] + rr // ratio if isinstance(rr, int)
                                    else uoff[t2] + lax.shift_right_logical(rr, _log2(ratio))]
                else:
                    kv_s = kv_sem.at[t2 % 2]
                start_kv(0, t2, t % 2, rr * hc, hc, kv_s)

            def refill_x():
                start_x(t2, t2 % NXS, u_sem.at[uoff[t2]] if t2 < kw else x_sem.at[t2 % 2])

            if t == 0:
                m = (cpi[1] + 1) // 2
                for rr in range(m):
                    @pl.when(r == rr)
                    def _(rr=rr):
                        for u in range(2 * rr, min(2 * rr + 2, cpi[1])):
                            start_unit(1, u)

                @pl.when(r == m)
                def _():
                    refill_x()
                    for rr in range(m):
                        refill(rr)

                @pl.when(r >= m)
                def _():
                    refill(r)
            else:
                @pl.when(r == 0)
                def _():
                    refill_x()

                refill(r)
            return carry

        lax.fori_loop(0, cpi[t], chunk, 0)

    def body(t, carry):
        g, bb = split(t)
        slot = jnp.bitwise_and(t, 1)
        xslot = jnp.bitwise_and(t, NXS - 1)
        gslot = jnp.bitwise_and(g, 1)
        last_g = g == ng - 1

        wait_total(x_buf.at[xslot], x_sem.at[slot])
        wait_total(kv_buf.at[slot], kv_sem.at[slot])

        @pl.when(jnp.logical_and(bb == 0, g > 0))
        def _():
            wait_total(wq_buf.at[gslot], wq_sem.at[gslot])
            wait_total(wo_buf.at[gslot], wo_sem.at[gslot])

        @pl.when(jnp.logical_and(last_g, bb >= 2))
        def _():
            o_copy(bb - 2, slot).wait()

        compute(xslot, slot, gslot, bb, 0, hg, g == 0, True)

        @pl.when(t + 2 < T)
        def _():
            g2, bb2 = split(t + 2)
            start_x(bb2, jnp.bitwise_and(t + 2, NXS - 1), x_sem.at[slot])
            start_kv(g2, bb2, slot, 0, hg, kv_sem.at[slot])

        jobs = ((wq_copy, wq_sem, 0), (wo_copy, wo_sem, 0), (wq_copy, wq_sem, 1), (wo_copy, wo_sem, 1))
        for j, (fn, sem, p) in enumerate(jobs):
            @pl.when(jnp.logical_and(bb == min(kw + j, nbb - 2), g + 1 < ng))
            def _(fn=fn, sem=sem, p=p):
                fn(g + 1, 1 - gslot, p, 0, hg, sem.at[1 - gslot]).start()

        @pl.when(last_g)
        def _():
            o_copy(bb, slot).start()

        return carry

    assert kw <= nbb - 2 and cpi[0] > (cpi[1] + 1) // 2
    lax.fori_loop(kw, T, body, 0)
    o_copy(nbb - 2, 0).wait()
    o_copy(nbb - 1, 1).wait()


def run(A_x, A_k_cache, A_v_cache, A_wq, A_wo, B_x, B_k_cache, B_v_cache, B_wq, B_wo, *,
        hg=8, nb=2, stages=(1, 2, 4)):
    any_spec = pl.BlockSpec(memory_space=pl.ANY)
    assert len(stages) >= 2 and all(stages[i] <= stages[i + 1] for i in range(len(stages) - 1))
    nunits = sum(hg // hc for hc in stages)
    return pl.pallas_call(
        functools.partial(_kernel, hg=hg, nb=nb, stages=tuple(stages)),
        in_specs=[any_spec] * 10,
        out_specs=any_spec,
        out_shape=jax.ShapeDtypeStruct((B, SQ, 2 * D), BF16),
        scratch_shapes=[
            pltpu.VMEM((NXS, 2, nb, SQ, D), BF16),
            pltpu.VMEM((2, 4, nb, hg, SK, DH), BF16),
            pltpu.VMEM((2, 2, D, hg * DH), BF16),
            pltpu.VMEM((2, 2, hg * DH, D), BF16),
            pltpu.VMEM((B, SQ, 2 * D), F32),
            pltpu.VMEM((2, nb, SQ, 2 * D), BF16),
            pltpu.SemaphoreType.DMA((nunits,)),
            pltpu.SemaphoreType.DMA((2,)),
            pltpu.SemaphoreType.DMA((2,)),
            pltpu.SemaphoreType.DMA((2,)),
            pltpu.SemaphoreType.DMA((2,)),
            pltpu.SemaphoreType.DMA((2,)),
        ],
        compiler_params=pltpu.CompilerParams(
            vmem_limit_bytes=110 * 1024 * 1024,
            disable_bounds_checks=True,
        ),
    )(A_x, A_k_cache, A_v_cache, A_wq, A_wo, B_x, B_k_cache, B_v_cache, B_wq, B_wo)


@jax.jit
def pallas_concat_heads__mha_block_cached__mha_block_cached__near_ridge_kernel(
        A_x, A_k_cache, A_v_cache, A_wq, A_wo, B_x, B_k_cache, B_v_cache, B_wq, B_wo):
    return run(A_x, A_k_cache, A_v_cache, A_wq, A_wo, B_x, B_k_cache, B_v_cache, B_wq, B_wo)
```

```python
import functools
import jax
import jax.numpy as jnp
from jax import lax
import jax.experimental.pallas as pl
import jax.experimental.pallas.tpu as pltpu

B, SQ, D = 16, 192, 512
H, SK, DH = 32, 512, 128
LOG2E = 1.4426950408889634
QSCALE = (DH ** -0.5) * LOG2E
F32 = jnp.float32
BF16 = jnp.bfloat16
NXS = 4


def _log2(n):
    assert n & (n - 1) == 0
    return n.bit_length() - 1


def _kernel(xa, ka, va, wqa, woa, xb, kb, vb, wqb, wob, o_hbm,
            x_buf, kv_buf, wq_buf, wo_buf, acc_ref, o_buf,
            u_sem, x_sem, kv_sem, wq_sem, wo_sem, o_sem, *, hg, nb, stages):
    ng = H // hg
    nbb = B // nb
    T = ng * nbb
    kw = len(stages)
    cpi = [hg // hc for hc in stages]
    uoff = [sum(cpi[:t]) for t in range(kw)]
    xs, ks, vs, wqs, wos = (xa, xb), (ka, kb), (va, vb), (wqa, wqb), (woa, wob)

    def split(t):
        return lax.shift_right_logical(t, _log2(nbb)), jnp.bitwise_and(t, nbb - 1)

    def wait_total(ref, sem):
        pltpu.make_async_copy(ref, ref, sem).wait()

    def start_x(bb, xslot, sem):
        for p in range(2):
            pltpu.make_async_copy(xs[p].at[pl.ds(bb * nb, nb)], x_buf.at[xslot, p], sem).start()

    def start_kv(gg, bb, sl, h0, nh, sem):
        for p in range(2):
            src = (pl.ds(bb * nb, nb), pl.ds(gg * hg + h0, nh))
            pltpu.make_async_copy(ks[p].at[src], kv_buf.at[sl, 2 * p, :, pl.ds(h0, nh)], sem).start()
            pltpu.make_async_copy(vs[p].at[src], kv_buf.at[sl, 2 * p + 1, :, pl.ds(h0, nh)], sem).start()

    def wq_start(gg, sl, p, h0, nh, sem):
        for h in range(nh):
            pltpu.make_async_copy(
                wqs[p].at[:, pl.ds(pl.multiple_of((gg * hg + h0 + h) * DH, DH), DH)],
                wq_buf.at[sl, p, h0 + h], sem).start()

    def wo_copy(gg, sl, p, h0, nh, sem):
        return pltpu.make_async_copy(
            wos[p].at[pl.ds(pl.multiple_of((gg * hg + h0) * DH, nh * DH), nh * DH), :],
            wo_buf.at[sl, p, pl.ds(pl.multiple_of(h0 * DH, nh * DH), nh * DH), :], sem)

    def wo_start(gg, sl, p, h0, nh, sem):
        wo_copy(gg, sl, p, h0, nh, sem).start()

    def o_copy(bb, sl):
        return pltpu.make_async_copy(o_buf.at[sl], o_hbm.at[pl.ds(bb * nb, nb)], o_sem.at[sl])

    def start_unit(t, r):
        hc = stages[t]
        sem = u_sem.at[uoff[t] + r]

        if isinstance(r, int):
            if r == 0:
                start_x(t, t % NXS, sem)
        else:
            @pl.when(r == 0)
            def _():
                start_x(t, t % NXS, sem)

        if t == 0:
            for p in range(2):
                wq_start(0, 0, p, r * hc, hc, sem)
        start_kv(0, t, t % 2, r * hc, hc, sem)
        if t == 0:
            for p in range(2):
                wo_copy(0, 0, p, r * hc, hc, sem).start()

    def wait_unit(t, r):
        hc = stages[t]
        sem = u_sem.at[uoff[t] + r]

        @pl.when(r == 0)
        def _():
            wait_total(x_buf.at[t % NXS], sem)

        if t == 0:
            cols = pl.ds(pl.multiple_of(r * (hc * DH), hc * DH), hc * DH)
            wait_total(wq_buf.at[0, :, pl.ds(r * hc, hc)], sem)
            wait_total(wo_buf.at[0, :, cols, :], sem)
        wait_total(kv_buf.at[t % 2, :, :, pl.ds(r * hc, hc)], sem)

    def compute(xslot, slot, gslot, bb, h0, nh, first_acc, write_out):
        heads = [(p, h) for p in range(2) for h in range(nh)]
        n = len(heads)
        q, s, o = {}, {}, {}

        def wcols(h):
            if isinstance(h0, int):
                return slice((h0 + h) * DH, (h0 + h + 1) * DH)
            return pl.ds(pl.multiple_of((h0 + h) * DH, DH), DH)

        def qproj(i):
            p, h = heads[i]
            x = x_buf[xslot, p].reshape(nb * SQ, D)
            qq = jnp.dot(x, wq_buf[gslot, p, h0 + h], preferred_element_type=F32)
            q[i] = (qq * QSCALE).astype(BF16)

        def qk(i, j):
            p, h = heads[i]
            s[i, j] = jax.lax.dot_general(q[i][j * SQ:(j + 1) * SQ], kv_buf[slot, 2 * p, j, h0 + h],
                                          (((1,), (1,)), ((), ())), preferred_element_type=F32)

        def pv(i, j):
            p, h = heads[i]
            sc = s.pop((i, j))
            m = jnp.max(sc, axis=-1, keepdims=True)
            e = jnp.exp2(sc - m)
            l = jnp.sum(e, axis=-1, keepdims=True)
            oo = jnp.dot(e.astype(BF16), kv_buf[slot, 2 * p + 1, j, h0 + h], preferred_element_type=F32)
            r = pl.reciprocal(l, approx=True)
            r = r * (2.0 - l * r)
            o[i, j] = (oo * r).astype(BF16)

        def out(i):
            p, h = heads[i]
            os_ = [o.pop((i, j)) for j in range(nb)]
            oc = jnp.concatenate(os_, axis=0) if nb > 1 else os_[0]
            d = jnp.dot(oc, wo_buf[gslot, p, wcols(h), :], preferred_element_type=F32)
            d = d.reshape(nb, SQ, D)
            prev = acc_ref[pl.ds(bb * nb, nb), :, p * D:(p + 1) * D]
            if h == 0:
                prev = jnp.where(first_acc, 0.0, prev)
            new = prev + d
            acc_ref[pl.ds(bb * nb, nb), :, p * D:(p + 1) * D] = new
            if write_out and h == nh - 1:
                o_buf[slot, :, :, p * D:(p + 1) * D] = new.astype(BF16)

        qproj(0)
        for i in range(n):
            for j in range(nb):
                qk(i, j)
            if i + 1 < n:
                qproj(i + 1)
            elif n > 1:
                out(i - 1)
            for j in range(nb):
                pv(i, j)
            if i != n - 2:
                out(i)

    def issue0(r, carry):
        start_unit(0, r)
        return carry

    lax.fori_loop(0, cpi[0], issue0, 0)

    for t in range(kw):
        hc = stages[t]

        def chunk(r, carry, t=t, hc=hc):
            wait_unit(t, r)
            compute(t % NXS, t % 2, 0, t, r * hc, hc, r == 0, False)

            t2 = t + 2

            def refill(rr):
                if t2 < kw:
                    ratio = stages[t2] // hc
                    kv_s = u_sem.at[uoff[t2] + rr // ratio if isinstance(rr, int)
                                    else uoff[t2] + lax.shift_right_logical(rr, _log2(ratio))]
                else:
                    kv_s = kv_sem.at[t2 % 2]
                start_kv(0, t2, t % 2, rr * hc, hc, kv_s)

            def refill_x():
                start_x(t2, t2 % NXS, u_sem.at[uoff[t2]] if t2 < kw else x_sem.at[t2 % 2])

            if t == 0:
                m = (cpi[1] + 1) // 2
                for rr in range(m):
                    @pl.when(r == rr)
                    def _(rr=rr):
                        for u in range(2 * rr, min(2 * rr + 2, cpi[1])):
                            start_unit(1, u)

                @pl.when(r == m)
                def _():
                    refill_x()
                    for rr in range(m):
                        refill(rr)

                @pl.when(r >= m)
                def _():
                    refill(r)
            else:
                @pl.when(r == 0)
                def _():
                    refill_x()

                refill(r)
            return carry

        lax.fori_loop(0, cpi[t], chunk, 0)

    def body(t, carry):
        g, bb = split(t)
        slot = jnp.bitwise_and(t, 1)
        xslot = jnp.bitwise_and(t, NXS - 1)
        gslot = jnp.bitwise_and(g, 1)
        last_g = g == ng - 1

        wait_total(x_buf.at[xslot], x_sem.at[slot])
        wait_total(kv_buf.at[slot], kv_sem.at[slot])

        @pl.when(jnp.logical_and(bb == 0, g > 0))
        def _():
            wait_total(wq_buf.at[gslot], wq_sem.at[gslot])
            wait_total(wo_buf.at[gslot], wo_sem.at[gslot])

        @pl.when(jnp.logical_and(last_g, bb >= 2))
        def _():
            o_copy(bb - 2, slot).wait()

        compute(xslot, slot, gslot, bb, 0, hg, g == 0, True)

        @pl.when(t + 2 < T)
        def _():
            g2, bb2 = split(t + 2)
            start_x(bb2, jnp.bitwise_and(t + 2, NXS - 1), x_sem.at[slot])
            start_kv(g2, bb2, slot, 0, hg, kv_sem.at[slot])

        jobs = ((wq_start, wq_sem, 0), (wo_start, wo_sem, 0), (wq_start, wq_sem, 1), (wo_start, wo_sem, 1))
        for j, (fn, sem, p) in enumerate(jobs):
            @pl.when(jnp.logical_and(bb == min(kw + j, nbb - 2), g + 1 < ng))
            def _(fn=fn, sem=sem, p=p):
                fn(g + 1, 1 - gslot, p, 0, hg, sem.at[1 - gslot])

        @pl.when(last_g)
        def _():
            o_copy(bb, slot).start()

        return carry

    assert kw <= nbb - 2 and cpi[0] > (cpi[1] + 1) // 2
    lax.fori_loop(kw, T, body, 0)
    o_copy(nbb - 2, 0).wait()
    o_copy(nbb - 1, 1).wait()


def run(A_x, A_k_cache, A_v_cache, A_wq, A_wo, B_x, B_k_cache, B_v_cache, B_wq, B_wo, *,
        hg=8, nb=2, stages=(1, 1, 4)):
    any_spec = pl.BlockSpec(memory_space=pl.ANY)
    assert len(stages) >= 2 and all(stages[i] <= stages[i + 1] for i in range(len(stages) - 1))
    nunits = sum(hg // hc for hc in stages)
    return pl.pallas_call(
        functools.partial(_kernel, hg=hg, nb=nb, stages=tuple(stages)),
        in_specs=[any_spec] * 10,
        out_specs=any_spec,
        out_shape=jax.ShapeDtypeStruct((B, SQ, 2 * D), BF16),
        scratch_shapes=[
            pltpu.VMEM((NXS, 2, nb, SQ, D), BF16),
            pltpu.VMEM((2, 4, nb, hg, SK, DH), BF16),
            pltpu.VMEM((2, 2, hg, D, DH), BF16),
            pltpu.VMEM((2, 2, hg * DH, D), BF16),
            pltpu.VMEM((B, SQ, 2 * D), F32),
            pltpu.VMEM((2, nb, SQ, 2 * D), BF16),
            pltpu.SemaphoreType.DMA((nunits,)),
            pltpu.SemaphoreType.DMA((2,)),
            pltpu.SemaphoreType.DMA((2,)),
            pltpu.SemaphoreType.DMA((2,)),
            pltpu.SemaphoreType.DMA((2,)),
            pltpu.SemaphoreType.DMA((2,)),
        ],
        compiler_params=pltpu.CompilerParams(
            vmem_limit_bytes=110 * 1024 * 1024,
            disable_bounds_checks=True,
        ),
    )(A_x, A_k_cache, A_v_cache, A_wq, A_wo, B_x, B_k_cache, B_v_cache, B_wq, B_wo)


@jax.jit
def pallas_concat_heads__mha_block_cached__mha_block_cached__near_ridge_kernel(
        A_x, A_k_cache, A_v_cache, A_wq, A_wo, B_x, B_k_cache, B_v_cache, B_wq, B_wo):
    return run(A_x, A_k_cache, A_v_cache, A_wq, A_wo, B_x, B_k_cache, B_v_cache, B_wq, B_wo)
```

```python
import functools

import jax
import jax.numpy as jnp
from jax import lax
import jax.experimental.pallas as pl
import jax.experimental.pallas.tpu as pltpu

B, SQ, D = 16, 192, 512
H, SK, DH = 32, 512, 128
LOG2E = 1.4426950408889634
QSCALE = (DH ** -0.5) * LOG2E
F32 = jnp.float32
BF16 = jnp.bfloat16

HG = 8
NB = 2
STAGES = (1, 1, 4)
NXS = 4


def _log2(n):
    assert n & (n - 1) == 0
    return n.bit_length() - 1


def _kernel(xa, ka, va, wqa, woa, xb, kb, vb, wqb, wob, o_hbm,
            x_buf, kv_buf, wq_buf, wo_buf, acc_ref, o_buf,
            u_sem, x_sem, kv_sem, wq_sem, wo_sem, o_sem, *, hg, nb, stages):
    ng = H // hg
    nbb = B // nb
    T = ng * nbb
    kw = len(stages)
    cpi = [hg // hc for hc in stages]
    uoff = [sum(cpi[:t]) for t in range(kw)]
    xs, ks, vs, wqs, wos = (xa, xb), (ka, kb), (va, vb), (wqa, wqb), (woa, wob)

    def split(t):
        return lax.shift_right_logical(t, _log2(nbb)), jnp.bitwise_and(t, nbb - 1)

    def wait_total(ref, sem):
        pltpu.make_async_copy(ref, ref, sem).wait()

    def start_x(bb, xslot, sem):
        for p in range(2):
            pltpu.make_async_copy(xs[p].at[pl.ds(bb * nb, nb)], x_buf.at[xslot, p], sem).start()

    def start_kv(gg, bb, sl, h0, nh, sem):
        for p in range(2):
            src = (pl.ds(bb * nb, nb), pl.ds(gg * hg + h0, nh))
            pltpu.make_async_copy(ks[p].at[src], kv_buf.at[sl, 2 * p, :, pl.ds(h0, nh)], sem).start()
            pltpu.make_async_copy(vs[p].at[src], kv_buf.at[sl, 2 * p + 1, :, pl.ds(h0, nh)], sem).start()

    def start_wq(gg, sl, p, h0, nh, sem):
        for h in range(nh):
            pltpu.make_async_copy(
                wqs[p].at[:, pl.ds(pl.multiple_of((gg * hg + h0 + h) * DH, DH), DH)],
                wq_buf.at[sl, p, h0 + h], sem).start()

    def start_wo(gg, sl, p, h0, nh, sem):
        pltpu.make_async_copy(
            wos[p].at[pl.ds(pl.multiple_of((gg * hg + h0) * DH, nh * DH), nh * DH), :],
            wo_buf.at[sl, p, pl.ds(pl.multiple_of(h0 * DH, nh * DH), nh * DH), :], sem).start()

    def o_copy(bb, sl, p):
        cols = pl.ds(p * D, D)
        return pltpu.make_async_copy(o_buf.at[sl, :, :, cols], o_hbm.at[pl.ds(bb * nb, nb), :, cols],
                                     o_sem.at[sl, p])

    def when_first(r, fn):
        if isinstance(r, int):
            if r == 0:
                fn()
        else:
            pl.when(r == 0)(fn)

    def start_unit(t, r):
        hc = stages[t]
        sem = u_sem.at[uoff[t] + r]
        when_first(r, lambda: start_x(t, t % NXS, sem))
        if t == 0:
            for p in range(2):
                start_wq(0, 0, p, r * hc, hc, sem)
        start_kv(0, t, t % 2, r * hc, hc, sem)
        if t == 0:
            for p in range(2):
                start_wo(0, 0, p, r * hc, hc, sem)

    def wait_unit(t, r):
        hc = stages[t]
        sem = u_sem.at[uoff[t] + r]
        when_first(r, lambda: wait_total(x_buf.at[t % NXS], sem))
        if t == 0:
            rows = pl.ds(pl.multiple_of(r * (hc * DH), hc * DH), hc * DH)
            wait_total(wq_buf.at[0, :, pl.ds(r * hc, hc)], sem)
            wait_total(wo_buf.at[0, :, rows, :], sem)
        wait_total(kv_buf.at[t % 2, :, :, pl.ds(r * hc, hc)], sem)

    def compute(xslot, slot, gslot, bb, h0, nh, first_acc, out_hook):
        heads = [(p, h) for p in range(2) for h in range(nh)]
        n = len(heads)
        q, s, o = {}, {}, {}

        def qproj(i):
            p, h = heads[i]
            x = x_buf[xslot, p].reshape(nb * SQ, D)
            qq = jnp.dot(x, wq_buf[gslot, p, h0 + h], preferred_element_type=F32)
            q[i] = (qq * QSCALE).astype(BF16)

        def qk(i, j):
            p, h = heads[i]
            s[i, j] = lax.dot_general(q[i][j * SQ:(j + 1) * SQ], kv_buf[slot, 2 * p, j, h0 + h],
                                      (((1,), (1,)), ((), ())), preferred_element_type=F32)

        def pv(i, j):
            p, h = heads[i]
            sc = s.pop((i, j))
            m = jnp.max(sc, axis=-1, keepdims=True)
            e = jnp.exp2(sc - m)
            l = jnp.sum(e, axis=-1, keepdims=True)
            oo = jnp.dot(e.astype(BF16), kv_buf[slot, 2 * p + 1, j, h0 + h], preferred_element_type=F32)
            r = pl.reciprocal(l, approx=True)
            r = r * (2.0 - l * r)
            o[i, j] = (oo * r).astype(BF16)

        def out(i):
            p, h = heads[i]
            if isinstance(h0, int):
                rows = slice((h0 + h) * DH, (h0 + h + 1) * DH)
            else:
                rows = pl.ds(pl.multiple_of((h0 + h) * DH, DH), DH)
            oc = jnp.concatenate([o.pop((i, j)) for j in range(nb)], axis=0)
            d = jnp.dot(oc, wo_buf[gslot, p, rows, :], preferred_element_type=F32).reshape(nb, SQ, D)
            prev = acc_ref[pl.ds(bb * nb, nb), :, p * D:(p + 1) * D]
            if h == 0:
                prev = jnp.where(first_acc, 0.0, prev)
            new = prev + d
            acc_ref[pl.ds(bb * nb, nb), :, p * D:(p + 1) * D] = new
            if out_hook is not None and h == nh - 1:
                o_buf[slot, :, :, p * D:(p + 1) * D] = new.astype(BF16)
                out_hook(p)

        qproj(0)
        for i in range(n):
            for j in range(nb):
                qk(i, j)
            if i + 1 < n:
                qproj(i + 1)
            else:
                out(i - 1)
            for j in range(nb):
                pv(i, j)
            if i != n - 2:
                out(i)

    def issue0(r, carry):
        start_unit(0, r)
        return carry

    lax.fori_loop(0, cpi[0], issue0, 0)

    for t in range(kw):
        def chunk(r, carry, t=t, hc=stages[t]):
            wait_unit(t, r)
            compute(t % NXS, t % 2, 0, t, r * hc, hc, r == 0, None)

            t2 = t + 2

            def refill(rr):
                if t2 < kw:
                    sh = _log2(stages[t2] // hc)
                    u = rr >> sh if isinstance(rr, int) else lax.shift_right_logical(rr, sh)
                    sem = u_sem.at[uoff[t2] + u]
                else:
                    sem = kv_sem.at[t2 % 2]
                start_kv(0, t2, t % 2, rr * hc, hc, sem)

            def refill_x():
                start_x(t2, t2 % NXS, u_sem.at[uoff[t2]] if t2 < kw else x_sem.at[t2 % 2])

            if t == 0:
                m = (cpi[1] + 1) // 2
                for rr in range(m):
                    @pl.when(r == rr)
                    def _(rr=rr):
                        for u in range(2 * rr, min(2 * rr + 2, cpi[1])):
                            start_unit(1, u)

                @pl.when(r == m)
                def _():
                    refill_x()
                    for rr in range(m):
                        refill(rr)

                @pl.when(r >= m)
                def _():
                    refill(r)
            else:
                pl.when(r == 0)(refill_x)
                refill(r)
            return carry

        lax.fori_loop(0, cpi[t], chunk, 0)

    def body(t, carry):
        g, bb = split(t)
        slot = jnp.bitwise_and(t, 1)
        xslot = jnp.bitwise_and(t, NXS - 1)
        gslot = jnp.bitwise_and(g, 1)
        last_g = g == ng - 1

        wait_total(x_buf.at[xslot], x_sem.at[slot])
        wait_total(kv_buf.at[slot], kv_sem.at[slot])

        @pl.when(jnp.logical_and(bb == 0, g > 0))
        def _():
            wait_total(wq_buf.at[gslot], wq_sem.at[gslot])
            wait_total(wo_buf.at[gslot], wo_sem.at[gslot])

        @pl.when(jnp.logical_and(last_g, bb >= 2))
        def _():
            for p in range(2):
                o_copy(bb - 2, slot, p).wait()

        def out_hook(p):
            @pl.when(last_g)
            def _():
                o_copy(bb, slot, p).start()

        compute(xslot, slot, gslot, bb, 0, hg, g == 0, out_hook)

        @pl.when(t + 2 < T)
        def _():
            g2, bb2 = split(t + 2)
            start_x(bb2, jnp.bitwise_and(t + 2, NXS - 1), x_sem.at[slot])
            start_kv(g2, bb2, slot, 0, hg, kv_sem.at[slot])

        jobs = ((start_wq, wq_sem, 0), (start_wo, wo_sem, 0), (start_wq, wq_sem, 1), (start_wo, wo_sem, 1))
        for j, (fn, sem, p) in enumerate(jobs):
            @pl.when(jnp.logical_and(bb == min(kw + j, nbb - 2), g + 1 < ng))
            def _(fn=fn, sem=sem, p=p):
                fn(g + 1, 1 - gslot, p, 0, hg, sem.at[1 - gslot])

        return carry

    lax.fori_loop(kw, T, body, 0)
    for p in range(2):
        o_copy(nbb - 2, 0, p).wait()
        o_copy(nbb - 1, 1, p).wait()


def run(A_x, A_k_cache, A_v_cache, A_wq, A_wo, B_x, B_k_cache, B_v_cache, B_wq, B_wo, *,
        hg=HG, nb=NB, stages=STAGES):
    nbb = B // nb
    kw = len(stages)
    assert 2 <= kw <= nbb - 2 and nbb % 2 == 0 and nb >= 2
    assert all(stages[i] <= stages[i + 1] for i in range(kw - 1))
    assert hg // stages[0] > (hg // stages[1] + 1) // 2
    any_spec = pl.BlockSpec(memory_space=pl.ANY)
    return pl.pallas_call(
        functools.partial(_kernel, hg=hg, nb=nb, stages=tuple(stages)),
        in_specs=[any_spec] * 10,
        out_specs=any_spec,
        out_shape=jax.ShapeDtypeStruct((B, SQ, 2 * D), BF16),
        scratch_shapes=[
            pltpu.VMEM((NXS, 2, nb, SQ, D), BF16),
            pltpu.VMEM((2, 4, nb, hg, SK, DH), BF16),
            pltpu.VMEM((2, 2, hg, D, DH), BF16),
            pltpu.VMEM((2, 2, hg * DH, D), BF16),
            pltpu.VMEM((B, SQ, 2 * D), F32),
            pltpu.VMEM((2, nb, SQ, 2 * D), BF16),
            pltpu.SemaphoreType.DMA((sum(hg // hc for hc in stages),)),
            pltpu.SemaphoreType.DMA((2,)),
            pltpu.SemaphoreType.DMA((2,)),
            pltpu.SemaphoreType.DMA((2,)),
            pltpu.SemaphoreType.DMA((2,)),
            pltpu.SemaphoreType.DMA((2, 2)),
        ],
        compiler_params=pltpu.CompilerParams(
            vmem_limit_bytes=100 * 1024 * 1024,
            disable_bounds_checks=True,
            disable_semaphore_checks=True,
        ),
    )(A_x, A_k_cache, A_v_cache, A_wq, A_wo, B_x, B_k_cache, B_v_cache, B_wq, B_wo)


@jax.jit
def pallas_concat_heads__mha_block_cached__mha_block_cached__near_ridge_kernel(
        A_x, A_k_cache, A_v_cache, A_wq, A_wo, B_x, B_k_cache, B_v_cache, B_wq, B_wo):
    return run(A_x, A_k_cache, A_v_cache, A_wq, A_wo, B_x, B_k_cache, B_v_cache, B_wq, B_wo)
```

```python
import functools

import jax
import jax.numpy as jnp
from jax import lax
import jax.experimental.pallas as pl
import jax.experimental.pallas.tpu as pltpu

B, SQ, D = 16, 192, 512
H, SK, DH = 32, 512, 128
LOG2E = 1.4426950408889634
QSCALE = (DH ** -0.5) * LOG2E
F32 = jnp.float32
BF16 = jnp.bfloat16

HG = 8
NB = 2
NS = 4
FH = 4
NG = H // HG
NBB = B // NB
T = NG * NBB
NFC = HG // FH


def _log2(n):
    assert n & (n - 1) == 0
    return n.bit_length() - 1


def _kernel(xa, ka, va, wqa, woa, xb, kb, vb, wqb, wob, o_hbm,
            x_buf, q_buf, kv_buf, wq_buf, wo_buf, acc_ref, o_buf,
            x_sem, kv_sem, wq_sem, wo_sem, o_sem, w0_sem):
    xs, ks, vs, wqs, wos = (xa, xb), (ka, kb), (va, vb), (wqa, wqb), (woa, wob)

    def split(t):
        return lax.shift_right_logical(t, _log2(NBB)), jnp.bitwise_and(t, NBB - 1)

    def wait_total(ref, sem):
        pltpu.make_async_copy(ref, ref, sem).wait()

    def x_copy(bb, p):
        rows = pl.ds(bb * NB, NB)
        return pltpu.make_async_copy(xs[p].at[rows], x_buf.at[p, rows], x_sem.at[bb, p])

    def start_kv(t):
        g, bb = split(t)
        sl = jnp.bitwise_and(t, NS - 1)
        src = (pl.ds(bb * NB, NB), pl.ds(g * HG, HG))
        for p in range(2):
            pltpu.make_async_copy(ks[p].at[src], kv_buf.at[sl, 2 * p], kv_sem.at[sl]).start()
            pltpu.make_async_copy(vs[p].at[src], kv_buf.at[sl, 2 * p + 1], kv_sem.at[sl]).start()

    def start_wq_tile(g, sl, p, h, sem):
        pltpu.make_async_copy(wqs[p].at[:, pl.ds(pl.multiple_of((g * HG + h) * DH, DH), DH)],
                              wq_buf.at[sl, p, h], sem).start()

    def start_wq(g, sl, p):
        for h in range(HG):
            start_wq_tile(g, sl, p, h, wq_sem.at[sl])

    def start_wo(g, sl, p):
        pltpu.make_async_copy(wos[p].at[pl.ds(pl.multiple_of(g * (HG * DH), HG * DH), HG * DH), :],
                              wo_buf.at[sl, p], wo_sem.at[sl]).start()

    def o_copy(bb, sl, p):
        cols = pl.ds(p * D, D)
        return pltpu.make_async_copy(o_buf.at[sl, :, :, cols], o_hbm.at[pl.ds(bb * NB, NB), :, cols],
                                     o_sem.at[sl, p])

    def load_x(p, bb, nblk=1):
        return x_buf[p, pl.ds(bb * NB, nblk * NB)].reshape(nblk * NB * SQ, D)

    def project(x, w):
        return (jnp.dot(x, w, preferred_element_type=F32) * QSCALE).astype(BF16)

    def attend(slot, oslot, gslot, bb, have_q, out_hook):
        heads = [(p, h) for p in range(2) for h in range(HG)]
        n = len(heads)
        q, s, o = {}, {}, {}

        def qproj(i):
            p, h = heads[i]
            q[i] = project(load_x(p, bb), wq_buf[gslot, p, h])

        def qk(i, j):
            p, h = heads[i]
            rows = slice(j * SQ, (j + 1) * SQ)
            qi = q_buf[bb, p, h, rows, :] if have_q else q[i][rows]
            s[i, j] = lax.dot_general(qi, kv_buf[slot, 2 * p, j, h],
                                      (((1,), (1,)), ((), ())), preferred_element_type=F32)

        def pv(i, j):
            p, h = heads[i]
            sc = s.pop((i, j))
            m = jnp.max(sc, axis=-1, keepdims=True)
            e = jnp.exp2(sc - m)
            l = jnp.sum(e, axis=-1, keepdims=True)
            oo = jnp.dot(e.astype(BF16), kv_buf[slot, 2 * p + 1, j, h], preferred_element_type=F32)
            r = pl.reciprocal(l, approx=True)
            r = r * (2.0 - l * r)
            o[i, j] = (oo * r).astype(BF16)

        def out(i):
            p, h = heads[i]
            oc = jnp.concatenate([o.pop((i, j)) for j in range(NB)], axis=0)
            d = jnp.dot(oc, wo_buf[gslot, p, h * DH:(h + 1) * DH, :],
                        preferred_element_type=F32).reshape(NB, SQ, D)
            dst = (pl.ds(bb * NB, NB), slice(None), slice(p * D, (p + 1) * D))
            new = d if (have_q and h == 0) else acc_ref[dst] + d
            acc_ref[dst] = new
            if out_hook is not None and h == HG - 1:
                o_buf[oslot, :, :, p * D:(p + 1) * D] = new.astype(BF16)
                out_hook(p)

        if have_q:
            qk(0, 0)
            qk(0, 1)
            for i in range(n):
                if i + 1 < n:
                    qk(i + 1, 0)
                pv(i, 0)
                if i >= 1:
                    out(i - 1)
                if i + 1 < n:
                    qk(i + 1, 1)
                pv(i, 1)
            out(n - 1)
        else:
            qproj(0)
            for i in range(n):
                qk(i, 0)
                qk(i, 1)
                if i + 1 < n:
                    qproj(i + 1)
                else:
                    out(i - 1)
                pv(i, 0)
                pv(i, 1)
                if i != n - 2:
                    out(i)

    for p in range(2):
        def issue_w(h, carry, p=p):
            @pl.when(h == 0)
            def _():
                x_copy(0, p).start()

            start_wq_tile(0, 0, p, h, w0_sem.at[p * NFC + lax.shift_right_logical(h, _log2(FH))])
            return carry

        lax.fori_loop(0, HG, issue_w, 0)

    def issue_x(bb, carry):
        for p in range(2):
            x_copy(bb, p).start()
        return carry

    lax.fori_loop(1, NBB, issue_x, 0)

    def issue_kv(t, carry):
        @pl.when(t == 0)
        def _():
            for p in range(2):
                start_wo(0, 0, p)

        start_kv(t)
        return carry

    lax.fori_loop(0, NS, issue_kv, 0)

    def q_first(c, carry):
        p = lax.shift_right_logical(c, _log2(NFC))
        h0 = jnp.bitwise_and(c, NFC - 1) * FH

        @pl.when(h0 == 0)
        def _():
            wait_total(x_buf.at[p, pl.ds(0, NB)], x_sem.at[0, p])

        wait_total(wq_buf.at[0, p, pl.ds(h0, FH)], w0_sem.at[c])
        x = load_x(p, 0)
        for h in range(FH):
            q_buf[0, p, h0 + h] = project(x, wq_buf[0, p, h0 + h])
        return carry

    lax.fori_loop(0, 2 * NFC, q_first, 0)

    def q_rest(nblk):
        def step(k, carry):
            bb = k * nblk
            for j in range(nblk):
                for p in range(2):
                    x_copy(bb + j, p).wait()
            for p in range(2):
                x = load_x(p, bb, nblk)
                for h in range(HG):
                    qq = project(x, wq_buf[0, p, h])
                    for j in range(nblk):
                        q_buf[bb + j, p, h] = qq[j * NB * SQ:(j + 1) * NB * SQ]
            return carry
        return step

    lax.fori_loop(1, 2, q_rest(1), 0)
    lax.fori_loop(1, NBB // 2, q_rest(2), 0)

    def prefetch(t, g, bb, gslot):
        jobs = ((start_wq, 0), (start_wo, 0), (start_wq, 1), (start_wo, 1))
        for j, (fn, p) in enumerate(jobs):
            @pl.when(jnp.logical_and(bb == 1 + j // 2, g + 1 < NG))
            def _(fn=fn, p=p):
                fn(g + 1, 1 - gslot, p)

        @pl.when(t + NS < T)
        def _():
            start_kv(t + NS)

    def body0(t, carry):
        slot = jnp.bitwise_and(t, NS - 1)
        wait_total(kv_buf.at[slot], kv_sem.at[slot])

        @pl.when(t == 0)
        def _():
            wait_total(wo_buf.at[0], wo_sem.at[0])

        attend(slot, None, 0, t, True, None)
        prefetch(t, 0, t, 0)
        return carry

    lax.fori_loop(0, NBB, body0, 0)

    def body(t, carry):
        g, bb = split(t)
        slot = jnp.bitwise_and(t, NS - 1)
        oslot = jnp.bitwise_and(t, 1)
        gslot = jnp.bitwise_and(g, 1)
        last_g = g == NG - 1

        wait_total(kv_buf.at[slot], kv_sem.at[slot])

        @pl.when(bb == 0)
        def _():
            wait_total(wq_buf.at[gslot], wq_sem.at[gslot])
            wait_total(wo_buf.at[gslot], wo_sem.at[gslot])

        @pl.when(jnp.logical_and(last_g, bb >= 2))
        def _():
            for p in range(2):
                o_copy(bb - 2, oslot, p).wait()

        def out_hook(p):
            @pl.when(last_g)
            def _():
                o_copy(bb, oslot, p).start()

        attend(slot, oslot, gslot, bb, False, out_hook)
        prefetch(t, g, bb, gslot)
        return carry

    lax.fori_loop(NBB, T, body, 0)
    for p in range(2):
        o_copy(NBB - 2, 0, p).wait()
        o_copy(NBB - 1, 1, p).wait()


def run(A_x, A_k_cache, A_v_cache, A_wq, A_wo, B_x, B_k_cache, B_v_cache, B_wq, B_wo):
    any_spec = pl.BlockSpec(memory_space=pl.ANY)
    return pl.pallas_call(
        _kernel,
        in_specs=[any_spec] * 10,
        out_specs=any_spec,
        out_shape=jax.ShapeDtypeStruct((B, SQ, 2 * D), BF16),
        scratch_shapes=[
            pltpu.VMEM((2, B, SQ, D), BF16),
            pltpu.VMEM((NBB, 2, HG, NB * SQ, DH), BF16),
            pltpu.VMEM((NS, 4, NB, HG, SK, DH), BF16),
            pltpu.VMEM((2, 2, HG, D, DH), BF16),
            pltpu.VMEM((2, 2, HG * DH, D), BF16),
            pltpu.VMEM((B, SQ, 2 * D), F32),
            pltpu.VMEM((2, NB, SQ, 2 * D), BF16),
            pltpu.SemaphoreType.DMA((NBB, 2)),
            pltpu.SemaphoreType.DMA((NS,)),
            pltpu.SemaphoreType.DMA((2,)),
            pltpu.SemaphoreType.DMA((2,)),
            pltpu.SemaphoreType.DMA((2, 2)),
            pltpu.SemaphoreType.DMA((2 * NFC,)),
        ],
        compiler_params=pltpu.CompilerParams(
            vmem_limit_bytes=110 * 1024 * 1024,
            disable_bounds_checks=True,
            disable_semaphore_checks=True,
        ),
    )(A_x, A_k_cache, A_v_cache, A_wq, A_wo, B_x, B_k_cache, B_v_cache, B_wq, B_wo)


@jax.jit
def pallas_concat_heads__mha_block_cached__mha_block_cached__near_ridge_kernel(
        A_x, A_k_cache, A_v_cache, A_wq, A_wo, B_x, B_k_cache, B_v_cache, B_wq, B_wo):
    return run(A_x, A_k_cache, A_v_cache, A_wq, A_wo, B_x, B_k_cache, B_v_cache, B_wq, B_wo)
```

```python
import jax
import jax.numpy as jnp
from jax import lax
import jax.experimental.pallas as pl
import jax.experimental.pallas.tpu as pltpu

B, SQ, D = 16, 192, 512
H, SK, DH = 32, 512, 128
LOG2E = 1.4426950408889634
QSCALE = (DH ** -0.5) * LOG2E
F32 = jnp.float32
BF16 = jnp.bfloat16

HG = 8
NB = 2
NS = 4
FH = 4
NG = H // HG
NBB = B // NB
T = NG * NBB
NFC = HG // FH


def _log2(n):
    assert n & (n - 1) == 0
    return n.bit_length() - 1


def _kernel(xa, ka, va, wqa, woa, xb, kb, vb, wqb, wob, o_hbm,
            x_buf, q_buf, kv_buf, wq_buf, wo_buf, acc_ref, o_buf,
            x_sem, kv_sem, wq_sem, wo_sem, o_sem, w0_sem):
    xs, ks, vs, wqs, wos = (xa, xb), (ka, kb), (va, vb), (wqa, wqb), (woa, wob)

    def split(t):
        return lax.shift_right_logical(t, _log2(NBB)), jnp.bitwise_and(t, NBB - 1)

    def wait_total(ref, sem):
        pltpu.make_async_copy(ref, ref, sem).wait()

    def x_copy(bb, p):
        rows = pl.ds(bb * NB, NB)
        return pltpu.make_async_copy(xs[p].at[rows], x_buf.at[p, rows], x_sem.at[bb, p])

    def start_kv(t):
        g, bb = split(t)
        sl = jnp.bitwise_and(t, NS - 1)
        src = (pl.ds(bb * NB, NB), pl.ds(g * HG, HG))
        for p in range(2):
            pltpu.make_async_copy(ks[p].at[src], kv_buf.at[sl, 2 * p], kv_sem.at[sl]).start()
            pltpu.make_async_copy(vs[p].at[src], kv_buf.at[sl, 2 * p + 1], kv_sem.at[sl]).start()

    def start_wq_tile(g, sl, p, h, sem):
        pltpu.make_async_copy(wqs[p].at[:, pl.ds(pl.multiple_of((g * HG + h) * DH, DH), DH)],
                              wq_buf.at[sl, p, h], sem).start()

    def start_wq(g, sl, p):
        for h in range(HG):
            start_wq_tile(g, sl, p, h, wq_sem.at[sl])

    def start_wo(g, sl, p):
        pltpu.make_async_copy(wos[p].at[pl.ds(pl.multiple_of(g * (HG * DH), HG * DH), HG * DH), :],
                              wo_buf.at[sl, p], wo_sem.at[sl]).start()

    def o_copy(bb, sl, p):
        cols = pl.ds(p * D, D)
        return pltpu.make_async_copy(o_buf.at[sl, :, :, cols], o_hbm.at[pl.ds(bb * NB, NB), :, cols],
                                     o_sem.at[sl, p])

    def load_x(p, bb, nblk=1):
        return x_buf[p, pl.ds(bb * NB, nblk * NB)].reshape(nblk * NB * SQ, D)

    def project(x, w):
        return (jnp.dot(x, w, preferred_element_type=F32) * QSCALE).astype(BF16)

    def attend(slot, oslot, gslot, bb, have_q, out_hook):
        heads = [(p, h) for p in range(2) for h in range(HG)]
        n = len(heads)
        q, s, o = {}, {}, {}

        def qproj(i):
            p, h = heads[i]
            q[i] = project(load_x(p, bb), wq_buf[gslot, p, h])

        def qk(i, j):
            p, h = heads[i]
            rows = slice(j * SQ, (j + 1) * SQ)
            qi = q_buf[bb, p, h, rows, :] if have_q else q[i][rows]
            s[i, j] = lax.dot_general(qi, kv_buf[slot, 2 * p, j, h],
                                      (((1,), (1,)), ((), ())), preferred_element_type=F32)

        def pv(i, j):
            p, h = heads[i]
            sc = s.pop((i, j))
            m = jnp.max(sc, axis=-1, keepdims=True)
            e = jnp.exp2(sc - m)
            l = jnp.sum(e, axis=-1, keepdims=True)
            oo = jnp.dot(e.astype(BF16), kv_buf[slot, 2 * p + 1, j, h], preferred_element_type=F32)
            r = pl.reciprocal(l, approx=True)
            r = r * (2.0 - l * r)
            o[i, j] = (oo * r).astype(BF16)

        def out(i):
            p, h = heads[i]
            oc = jnp.concatenate([o.pop((i, j)) for j in range(NB)], axis=0)
            d = jnp.dot(oc, wo_buf[gslot, p, h * DH:(h + 1) * DH, :],
                        preferred_element_type=F32).reshape(NB, SQ, D)
            dst = (pl.ds(bb * NB, NB), slice(None), slice(p * D, (p + 1) * D))
            new = acc_ref[dst] + d
            acc_ref[dst] = new
            if h == HG - 1:
                o_buf[oslot, :, :, p * D:(p + 1) * D] = new.astype(BF16)
                out_hook(p)

        pair = {}

        def out_pair(i, half):
            p, h = heads[i]
            if half == 0:
                pair[i] = jnp.concatenate(
                    [jnp.concatenate([o.pop((ii, j)) for j in range(NB)], axis=0) for ii in (i - 1, i)],
                    axis=1)
            oc = pair[i] if half == 0 else pair.pop(i)
            c0 = half * (D // 2)
            d = jnp.dot(oc, wo_buf[gslot, p, (h - 1) * DH:(h + 1) * DH, c0:c0 + D // 2],
                        preferred_element_type=F32).reshape(NB, SQ, D // 2)
            dst = (pl.ds(bb * NB, NB), slice(None), slice(p * D + c0, p * D + c0 + D // 2))
            acc_ref[dst] = d if h == 1 else acc_ref[dst] + d

        if have_q:
            qk(0, 0)
            qk(0, 1)
            for i in range(n):
                if i + 1 < n:
                    qk(i + 1, 0)
                pv(i, 0)
                if i >= 2:
                    if i % 2 == 0:
                        out_pair(i - 1, 0)
                    else:
                        out_pair(i - 2, 1)
                if i + 1 < n:
                    qk(i + 1, 1)
                pv(i, 1)
            out_pair(n - 1, 0)
            out_pair(n - 1, 1)
        else:
            qproj(0)
            for i in range(n):
                qk(i, 0)
                qk(i, 1)
                if i + 1 < n:
                    qproj(i + 1)
                else:
                    out(i - 1)
                pv(i, 0)
                pv(i, 1)
                if i != n - 2:
                    out(i)

    for p in range(2):
        def issue_w(h, carry, p=p):
            @pl.when(h == 0)
            def _():
                x_copy(0, p).start()

            start_wq_tile(0, 0, p, h, w0_sem.at[p * NFC + lax.shift_right_logical(h, _log2(FH))])
            return carry

        lax.fori_loop(0, HG, issue_w, 0)

    def issue_x(bb, carry):
        for p in range(2):
            x_copy(bb, p).start()
        return carry

    lax.fori_loop(1, NBB, issue_x, 0)

    def issue_kv(t, carry):
        @pl.when(t == 0)
        def _():
            for p in range(2):
                start_wo(0, 0, p)

        start_kv(t)
        return carry

    lax.fori_loop(0, NS, issue_kv, 0)

    def q_first(c, carry):
        p = lax.shift_right_logical(c, _log2(NFC))
        h0 = jnp.bitwise_and(c, NFC - 1) * FH

        @pl.when(h0 == 0)
        def _():
            wait_total(x_buf.at[p, pl.ds(0, NB)], x_sem.at[0, p])

        wait_total(wq_buf.at[0, p, pl.ds(h0, FH)], w0_sem.at[c])
        x = load_x(p, 0)
        for h in range(FH):
            q_buf[0, p, h0 + h] = project(x, wq_buf[0, p, h0 + h])
        return carry

    lax.fori_loop(0, 2 * NFC, q_first, 0)

    def q_rest(nblk):
        def step(k, carry):
            bb = k * nblk
            for j in range(nblk):
                for p in range(2):
                    x_copy(bb + j, p).wait()
            for p in range(2):
                x = load_x(p, bb, nblk)
                for h in range(HG):
                    qq = project(x, wq_buf[0, p, h])
                    for j in range(nblk):
                        q_buf[bb + j, p, h] = qq[j * NB * SQ:(j + 1) * NB * SQ]
            return carry
        return step

    lax.fori_loop(1, 2, q_rest(1), 0)
    lax.fori_loop(1, NBB // 2, q_rest(2), 0)

    def prefetch(t, g, bb, gslot):
        jobs = ((start_wq, 0), (start_wo, 0), (start_wq, 1), (start_wo, 1))
        for j, (fn, p) in enumerate(jobs):
            @pl.when(jnp.logical_and(bb == 1 + j // 2, g + 1 < NG))
            def _(fn=fn, p=p):
                fn(g + 1, 1 - gslot, p)

        @pl.when(t + NS < T)
        def _():
            start_kv(t + NS)

    def body0(t, carry):
        slot = jnp.bitwise_and(t, NS - 1)
        wait_total(kv_buf.at[slot], kv_sem.at[slot])

        @pl.when(t == 0)
        def _():
            wait_total(wo_buf.at[0], wo_sem.at[0])

        attend(slot, None, 0, t, True, None)
        prefetch(t, 0, t, 0)
        return carry

    lax.fori_loop(0, NBB, body0, 0)

    def body(t, carry):
        g, bb = split(t)
        slot = jnp.bitwise_and(t, NS - 1)
        oslot = jnp.bitwise_and(t, 1)
        gslot = jnp.bitwise_and(g, 1)
        last_g = g == NG - 1

        wait_total(kv_buf.at[slot], kv_sem.at[slot])

        @pl.when(bb == 0)
        def _():
            wait_total(wq_buf.at[gslot], wq_sem.at[gslot])
            wait_total(wo_buf.at[gslot], wo_sem.at[gslot])

        @pl.when(jnp.logical_and(last_g, bb >= 2))
        def _():
            for p in range(2):
                o_copy(bb - 2, oslot, p).wait()

        def out_hook(p):
            @pl.when(last_g)
            def _():
                o_copy(bb, oslot, p).start()

        attend(slot, oslot, gslot, bb, False, out_hook)
        prefetch(t, g, bb, gslot)
        return carry

    lax.fori_loop(NBB, T, body, 0)
    for p in range(2):
        o_copy(NBB - 2, 0, p).wait()
        o_copy(NBB - 1, 1, p).wait()


def run(A_x, A_k_cache, A_v_cache, A_wq, A_wo, B_x, B_k_cache, B_v_cache, B_wq, B_wo):
    any_spec = pl.BlockSpec(memory_space=pl.ANY)
    return pl.pallas_call(
        _kernel,
        in_specs=[any_spec] * 10,
        out_specs=any_spec,
        out_shape=jax.ShapeDtypeStruct((B, SQ, 2 * D), BF16),
        scratch_shapes=[
            pltpu.VMEM((2, B, SQ, D), BF16),
            pltpu.VMEM((NBB, 2, HG, NB * SQ, DH), BF16),
            pltpu.VMEM((NS, 4, NB, HG, SK, DH), BF16),
            pltpu.VMEM((2, 2, HG, D, DH), BF16),
            pltpu.VMEM((2, 2, HG * DH, D), BF16),
            pltpu.VMEM((B, SQ, 2 * D), F32),
            pltpu.VMEM((2, NB, SQ, 2 * D), BF16),
            pltpu.SemaphoreType.DMA((NBB, 2)),
            pltpu.SemaphoreType.DMA((NS,)),
            pltpu.SemaphoreType.DMA((2,)),
            pltpu.SemaphoreType.DMA((2,)),
            pltpu.SemaphoreType.DMA((2, 2)),
            pltpu.SemaphoreType.DMA((2 * NFC,)),
        ],
        compiler_params=pltpu.CompilerParams(
            vmem_limit_bytes=110 * 1024 * 1024,
            disable_bounds_checks=True,
            disable_semaphore_checks=True,
        ),
    )(A_x, A_k_cache, A_v_cache, A_wq, A_wo, B_x, B_k_cache, B_v_cache, B_wq, B_wo)


@jax.jit
def pallas_concat_heads__mha_block_cached__mha_block_cached__near_ridge_kernel(
        A_x, A_k_cache, A_v_cache, A_wq, A_wo, B_x, B_k_cache, B_v_cache, B_wq, B_wo):
    return run(A_x, A_k_cache, A_v_cache, A_wq, A_wo, B_x, B_k_cache, B_v_cache, B_wq, B_wo)
```
